```python
import os as _os
_os.environ.setdefault("JAX_PLATFORMS", "cpu")
import jax
import jax.numpy as jnp

def _softmax(x, axis=-1):
    return jax.nn.softmax(x, axis=axis)
def _gelu(x):
    return jax.nn.gelu(x, approximate=True)
def _silu(x):
    return jax.nn.silu(x)
def _sigmoid(x):
    return jax.nn.sigmoid(x)
def _layernorm(x, axis=-1, eps=1e-5):
    m = jnp.mean(x, axis=axis, keepdims=True)
    v = jnp.var(x, axis=axis, keepdims=True)
    return (x - m) / jnp.sqrt(v + eps)
def _scatter_add(tgt, idx, src, axis=0):
    return tgt.at[idx].add(src)
def _segment_sum(src, seg, n):
    return jax.ops.segment_sum(src, seg, n)
class _Rng:
    def __init__(self, key):
        self._k = key
    def _next(self):
        self._k, sub = jax.random.split(self._k)
        return sub
    def normal(self, shape):
        return jax.random.normal(self._next(), shape, dtype=jnp.bfloat16)
    def randint(self, lo, hi, shape):
        return jax.random.randint(self._next(), shape, lo, hi, dtype=jnp.int32)
    def uniform(self, shape, lo=0.0, hi=1.0):
        return jax.random.uniform(self._next(), shape, jnp.bfloat16, lo, hi)
    def permutation(self, n):
        return jax.random.permutation(self._next(), n)


kernel_name = 'gated_mix__linear_attn_block__glu_gated_swiglu__prompt'

def setup_inputs():
    _rng = _Rng(jax.random.key(int.from_bytes(__import__("os").urandom(4), "little")))
    _w = (lambda a: (lambda t: t.astype(jnp.bfloat16) if jnp.issubdtype(t.dtype, jnp.floating) else t)(jnp.asarray(a)))
    def _A_setup():
        B, S, D = 1, 2048, 1024
        return {
            "x": _w((lambda *s: _rng.normal(s) * 0.05)(B, S, D)),
            "wqkv": _w((lambda *s: _rng.normal(s) * 0.8)(D, 3 * D)),
            "wo": _w((lambda *s: _rng.normal(s) * 0.05)(D, D)),
        }
    _A_in = _A_setup()

    def _B_setup():
        B, S, D, F = 1, 2048, 1024, 3584
        return {
            "x": _w((lambda *s: _rng.normal(s) * 0.05)(B, S, D)),
            "w1": _w((lambda *s: _rng.normal(s) * 1.6)(D, F) * (2.0 / D) ** 0.5),
            "w3": _w((lambda *s: _rng.normal(s) * 1.6)(D, F) * (2.0 / D) ** 0.5),
            "w2": _w((lambda *s: _rng.normal(s) * 1.6)(F, D) * (2.0 / F) ** 0.5),
        }
    _B_in = _B_setup()

    return {
        "A_x": _A_in["x"],
        "A_wqkv": _A_in["wqkv"],
        "A_wo": _A_in["wo"],
        "B_x": _B_in["x"],
        "B_w1": _B_in["w1"],
        "B_w3": _B_in["w3"],
        "B_w2": _B_in["w2"],
        "gate_w": _w((lambda *s: _rng.normal(s) * 0.05)(1024) * 16.0),
    }

def reference(A_x, A_wqkv, A_wo, B_x, B_w1, B_w3, B_w2, gate_w):
    def _A_ref(x, wqkv, wo):
        B, S, D = x.shape
        H = 32; Dh = D // H
        qkv = (lambda x, *d: x.transpose(*d))((x @ wqkv).reshape(B, S, 3, H, Dh), 2, 0, 3, 1, 4)
        q, k, v = qkv[0], qkv[1], qkv[2]
        phi = lambda t: jnp.where(t > 0, t + 1, jnp.exp(t)) + 1e-6
        pq, pk = phi(q), phi(k)
        kv = jnp.einsum("bhsd,bhse->bhde", pk, v)
        z = jnp.einsum("bhsd->bhd", pk)
        num = jnp.einsum("bhqd,bhde->bhqe", pq, kv)
        den = jnp.einsum("bhqd,bhd->bhq", pq, z)[..., None] + 1e-6
        o = num / den
        return (lambda x, *d: x.transpose(*d))(o, 0, 2, 1, 3).reshape(B, S, D) @ wo

    def _B_ref(x, w1, w3, w2):
        gate = jnp.einsum("bsd,df->bsf", x, w1)
        up = jnp.einsum("bsd,df->bsf", x, w3)
        h = _silu(gate) * up
        out = jnp.einsum("bsf,fd->bsd", h, w2)
        return out

    x = A_x
    g = _sigmoid((x * gate_w).sum(-1, keepdims=True))
    a = _A_ref(x, A_wqkv, A_wo)
    b = _B_ref(x, B_w1, B_w3, B_w2)
    return g * a + (1 - g) * b
```

```python
import os
import jax
import jax.numpy as jnp
from jax import lax
import jax.experimental.pallas as pl
import jax.experimental.pallas.tpu as pltpu

E = os.environ.get
TM = int(E("TM", 256))
TF = int(E("TF", 512))
TM1 = int(E("TM1", 256))
CW = int(E("CW", 256))
ORDER = E("ORDER", "B")
SIG = E("SIG", "tanh")
RECIP = E("RECIP", "nofull")
P1MODE = E("P1MODE", "peel")
DMAFIRST = int(E("DMAFIRST", 0))
XORD = int(E("XORD", 0))
QT = int(E("QT", 1))
QTT = int(E("QTT", 0))
QTPOS = int(E("QTPOS", 0))
GW2D = int(E("GW2D", 0))

import contextlib
SCOPES = int(E("SCOPES", 0))
def scope(n):
    return jax.named_scope(n) if SCOPES else contextlib.nullcontext()

S, D, F, H = 2048, 1024, 3584, 32
DH = D // H
NF = F // TF
NB = S // TM
NB1 = S // TM1
NJ = D // 128
f32 = jnp.float32
bf16 = jnp.bfloat16


def _phi(t):
    return jnp.where(t > 0, t + 1.0, jnp.exp(t)) + 1e-6


def _dot(a, b):
    return jnp.dot(a, b, preferred_element_type=f32)


def _recip(x):
    if RECIP == "div":
        return 1.0 / x
    if RECIP == "approx":
        return pltpu.reciprocal(x, approx=True)
    return pltpu.reciprocal(x, approx=False, full_range=False)


def _sigmoid(x):
    if SIG == "exp":
        return jax.nn.sigmoid(x)
    return 0.5 * jnp.tanh(0.5 * x) + 0.5


def _swiglu(gate, up, og):
    if SIG == "exp":
        return gate * jax.nn.sigmoid(gate) * up * og
    hg = 0.5 * gate
    return (hg * jnp.tanh(hg) + hg) * (up * og)


def _kernel(x_hbm, wqkv_hbm, wo_hbm, w1_hbm, w3_hbm, w2_hbm, gw_hbm, out_hbm,
            x_v, wq_v, wk_v, wv_v, wo_v, w1_v, w3_v, w2_v, m_v, kv_v, zb_v, out_v, gw_v, wqT_v, zc_v, sems, osems):
    nsem = [NB1]

    def cp(src, dst):
        i = nsem[0]
        nsem[0] += 1
        return pltpu.make_async_copy(src, dst, sems.at[i])

    ns = D // CW
    def xcopy(i):
        r = pl.ds(pl.multiple_of(i * TM1, TM1), TM1)
        return pltpu.make_async_copy(x_hbm.at[r], x_v.at[r], sems.at[i])
    x0 = xcopy(0)
    wk = [cp(wqkv_hbm.at[:, pl.ds(D + s * CW, CW)], wk_v.at[s]) for s in range(ns)]
    wv = [cp(wqkv_hbm.at[:, pl.ds(2 * D + s * CW, CW)], wv_v.at[s]) for s in range(ns)]
    gwc = cp(gw_hbm, gw_v)
    wo = cp(wo_hbm, wo_v)
    wq = cp(wqkv_hbm.at[:, pl.ds(0, D)], wq_v)
    ffn = []
    for f in range(NF):
        ffn.append(cp(w1_hbm.at[:, pl.ds(f * TF, TF)], w1_v.at[f]))
        ffn.append(cp(w3_hbm.at[:, pl.ds(f * TF, TF)], w3_v.at[f]))
        ffn.append(cp(w2_hbm.at[pl.ds(f * TF, TF)], w2_v.at[f]))
    xs = [xcopy(i) for i in range(1, NB1)]
    if XORD == 0:
        first = [x0] + wk + wv + xs
        rest = [gwc, wo, wq] + ffn
    elif XORD == 1:
        first = [x0] + wk + [xs[0]] + wv + xs[1:]
        rest = [gwc, wo, wq] + ffn
    else:
        first = [x0] + wk + wv + [xs[0]]
        rest = xs[1:] + [gwc, wo, wq] + ffn
    for c in first:
        c.start()
    if DMAFIRST == 0:
        for c in rest:
            c.start()

    def kv_update(pk, v, first):
        for j in range(NJ):
            sl = slice(j * 128, (j + 1) * 128)
            u = lax.dot_general(pk[:, sl], v[:, sl], (((0,), (0,)), ((), ())), preferred_element_type=f32)
            if first:
                kv_v[j] = u
            else:
                kv_v[j] += u

    def p1_first():
        x0.wait()
        xi = x_v[pl.ds(0, TM1), :]
        pks, vs = [], []
        for s in range(ns):
            wk[s].wait()
            if DMAFIRST == 2 and s == 0:
                for c in rest:
                    c.start()
            pks.append(_phi(_dot(xi, wk_v[s])).astype(bf16))
        for s in range(ns):
            wv[s].wait()
            if DMAFIRST == 1 and s == ns - 1:
                for c in rest:
                    c.start()
            vs.append(_dot(xi, wv_v[s]).astype(bf16))
        pk = jnp.concatenate(pks, axis=1)
        v = jnp.concatenate(vs, axis=1)
        kv_update(pk, v, True)
        return jnp.sum(pk.astype(f32), axis=0, keepdims=True)

    def p1(xi, z):
        pk = jnp.concatenate([_phi(_dot(xi, wk_v[s])).astype(bf16) for s in range(ns)], axis=1)
        v = jnp.concatenate([_dot(xi, wv_v[s]).astype(bf16) for s in range(ns)], axis=1)
        kv_update(pk, v, False)
        return z + jnp.sum(pk.astype(f32), axis=0, keepdims=True)

    with scope("A_p1first"):
        z = p1_first()
    if DMAFIRST == 3:
        for c in rest:
            c.start()
    if P1MODE == "unroll":
        for i in range(1, NB1):
            xs[i - 1].wait()
            z = p1(x_v[pl.ds(i * TM1, TM1), :], z)
    else:
        with scope("C_p1loop"):
            def p1body(i, z):
                xcopy(i).wait()
                return p1(x_v[pl.ds(pl.multiple_of(i * TM1, TM1), TM1), :], z)
            z = lax.fori_loop(1, NB1, p1body, z)

    with scope("D_wowait"):
        wo.wait()
        if QT:
            wq.wait()
    r_id = lax.broadcasted_iota(jnp.int32, (128, 128), 0) // DH
    c_id = lax.broadcasted_iota(jnp.int32, (128, 128), 1) // DH
    mask = r_id == c_id
    for j in range(NJ):
        sl = slice(j * 128, (j + 1) * 128)
        kvb = jnp.where(mask, kv_v[j], 0.0).astype(bf16)
        m_v[sl, :] = _dot(kvb, wo_v[sl, :]).astype(bf16)
        if QT:
            zc_v[sl, :] = jnp.broadcast_to(z[:, sl], (128, 128)).T
        else:
            zb_v[j] = jnp.where(mask, jnp.broadcast_to(z[:, sl], (128, 128)), 0.0).astype(bf16)

    if QT and QTPOS == 0:
        wqT_v[...] = wq_v[...].T
    with scope("E_restwait"):
        if not QT:
            wq.wait()
        gwc.wait()
        for c in ffn:
            c.wait()

    gw = gw_v[...].astype(f32).reshape(1, D)

    def ocopy(i, slot):
        return pltpu.make_async_copy(out_v.at[slot], out_hbm.at[pl.ds(pl.multiple_of(i * TM, TM), TM)], osems.at[slot])

    jsched = [[] for _ in range(NF)]
    for j in range(NJ):
        jsched[min(j * NF // NJ, NF - 1)].append(j)

    def p2(i, _):
        slot = i % 2

        @pl.when(i >= 2)
        def _():
            ocopy(i - 2, slot).wait()

        xi = x_v[pl.ds(pl.multiple_of(i * TM, TM), TM), :]
        g = _sigmoid(jnp.sum(xi.astype(f32) * gw, axis=-1, keepdims=True))
        og = 1.0 - g
        if QT:
            pqT = _phi(lax.dot_general(wqT_v[...], xi, (((1,), (1,)), ((), ())), preferred_element_type=f32))
        else:
            pq = _phi(_dot(xi, wq_v[...]))
            pqb = pq.astype(bf16)
        pqn = [None] * NJ
        acc = None
        hs = []
        for f in range(NF):
            dens = []
            for j in ([] if QT else jsched[f]):
                sl = slice(j * 128, (j + 1) * 128)
                dens.append(lax.dot_general(pqb[:, sl], zb_v[j], (((1,), (1,)), ((), ())), preferred_element_type=f32))
            gate = _dot(xi, w1_v[f])
            up = _dot(xi, w3_v[f])
            if ORDER == "B" and f > 0:
                d = _dot(hs[f - 1], w2_v[f - 1])
                acc = d if acc is None else acc + d
            for j, den in zip(jsched[f], dens):
                sl = slice(j * 128, (j + 1) * 128)
                pqn[j] = (pq[:, sl] * (g * _recip(den + 1e-6))).astype(bf16)
            if QT:
                for j in jsched[f]:
                    pj = pqT[j * 128:(j + 1) * 128, :]
                    zc = zc_v[j * 128:(j + 1) * 128, :]
                    t = pj * jnp.concatenate([zc] * (TM // 128), axis=1)
                    if QT == 1:
                        den = jnp.sum(t.reshape(4, DH, TM), axis=1, keepdims=True)
                    else:
                        den = jnp.sum(jnp.sum(t.reshape(4, DH // 8, 8, TM), axis=1), axis=1, keepdims=True)
                    r = _recip(den + 1e-6)
                    pqn[j] = (pj.reshape(4, DH, TM) * r).reshape(128, TM).astype(bf16)
            hs.append(_swiglu(gate, up, og).astype(bf16))
        if QT:
            pqcT = jnp.concatenate(pqn, axis=0)
            if QTT:
                A_term = lambda: g * _dot(pqcT.T, m_v[...])
            else:
                A_term = lambda: g * lax.dot_general(pqcT, m_v[...], (((0,), (0,)), ((), ())), preferred_element_type=f32)
        else:
            pqc = jnp.concatenate(pqn, axis=1)
            A_term = lambda: _dot(pqc, m_v[...])
        if ORDER == "B":
            acc = acc + A_term()
            acc = acc + _dot(hs[NF - 1], w2_v[NF - 1])
        else:
            for f in range(NF - 1):
                d = _dot(hs[f], w2_v[f])
                acc = d if acc is None else acc + d
            acc = acc + A_term()
            acc = acc + _dot(hs[NF - 1], w2_v[NF - 1])

        out_v[slot] = acc.astype(bf16)
        ocopy(i, slot).start()

    def p2s(i, c):
        with scope("Fi_iter"):
            return p2(i, c)
    with scope("F_p2"):
        lax.fori_loop(0, NB, p2s, None)
    with scope("G_tail"):
        ocopy(NB - 2, (NB - 2) % 2).wait()
        ocopy(NB - 1, (NB - 1) % 2).wait()


@jax.jit
def pallas_gated_mix__linear_attn_block__glu_gated_swiglu__prompt_kernel(
    A_x, A_wqkv, A_wo, B_x, B_w1, B_w3, B_w2, gate_w,
):
    del B_x
    any_spec = pl.BlockSpec(memory_space=pl.ANY)
    ns = D // CW
    out = pl.pallas_call(
        _kernel,
        out_shape=jax.ShapeDtypeStruct((S, D), bf16),
        in_specs=[any_spec] * 7,
        out_specs=any_spec,
        scratch_shapes=[
            pltpu.VMEM((S, D), bf16),
            pltpu.VMEM((D, D), bf16),
            pltpu.VMEM((ns, D, CW), bf16),
            pltpu.VMEM((ns, D, CW), bf16),
            pltpu.VMEM((D, D), bf16),
            pltpu.VMEM((NF, D, TF), bf16),
            pltpu.VMEM((NF, D, TF), bf16),
            pltpu.VMEM((NF, TF, D), bf16),
            pltpu.VMEM((D, D), bf16),
            pltpu.VMEM((NJ, 128, 128), f32),
            pltpu.VMEM((NJ, 128, 128), bf16),
            pltpu.VMEM((2, TM, D), bf16),
            pltpu.VMEM((1, D) if GW2D else (D,), bf16),
            pltpu.VMEM((D, D), bf16),
            pltpu.VMEM((D, 128), f32),
            pltpu.SemaphoreType.DMA((NB1 + 3 + 2 * ns + 3 * NF,)),
            pltpu.SemaphoreType.DMA((2,)),
        ],
        compiler_params=pltpu.CompilerParams(vmem_limit_bytes=110 * 1024 * 1024),
    )(A_x.reshape(S, D), A_wqkv, A_wo, B_w1, B_w3, B_w2, gate_w.reshape(1, D) if GW2D else gate_w)
    return out.reshape(1, S, D)
```

```python
import jax
import jax.numpy as jnp
from jax import lax
import jax.experimental.pallas as pl
import jax.experimental.pallas.tpu as pltpu

S, D, F, H = 2048, 1024, 3584, 32
DH = D // H
TM1 = 256
SLABS = (128, 128, 256, 512)
TM = 256
TF = 896
QPOS = 1
OSPLIT = 4

NF = F // TF
NB = S // TM
NB1 = S // TM1
NJ = D // 128
OW = D // OSPLIT
f32 = jnp.float32
bf16 = jnp.bfloat16


def _phi(t):
    return jnp.where(t > 0, t + 1.0, jnp.exp(t)) + 1e-6


def _dot(a, b):
    return jnp.dot(a, b, preferred_element_type=f32)


def _dot_tn(a, b):
    return lax.dot_general(a, b, (((0,), (0,)), ((), ())), preferred_element_type=f32)


def _dot_nt(a, b):
    return lax.dot_general(a, b, (((1,), (1,)), ((), ())), preferred_element_type=f32)


def _sigmoid(t):
    return 0.5 * jnp.tanh(0.5 * t) + 0.5


def _kernel(x_hbm, wqkv_hbm, wo_hbm, w1_hbm, w3_hbm, w2_hbm, gw_hbm, out_hbm,
            x_v, wq_v, wk_v, wv_v, wo_v, w1_v, w3_v, w2_v, gw_v,
            px_v, m_v, wqt_v, zc_v, out_v, sems, osems):
    def xcopy(i):
        r = pl.ds(pl.multiple_of(i * TM1, TM1), TM1)
        return pltpu.make_async_copy(x_hbm.at[r], x_v.at[r], sems.at[i])

    offs = [sum(SLABS[:s]) for s in range(len(SLABS))]
    wk = [pltpu.make_async_copy(wqkv_hbm.at[:, pl.ds(D + o, w)], wk_v.at[:, pl.ds(o, w)], sems.at[NB1 + s])
          for s, (o, w) in enumerate(zip(offs, SLABS))]
    sem_a = sems.at[NB1 + len(SLABS)]
    sem_b = sems.at[NB1 + len(SLABS) + 1]
    grp_a = [pltpu.make_async_copy(wqkv_hbm.at[:, pl.ds(2 * D, D)], wv_v, sem_a),
             pltpu.make_async_copy(wo_hbm, wo_v, sem_a),
             pltpu.make_async_copy(wqkv_hbm.at[:, pl.ds(0, D)], wq_v, sem_a)]
    grp_b = [pltpu.make_async_copy(gw_hbm, gw_v, sem_b),
             pltpu.make_async_copy(w1_hbm, w1_v, sem_b),
             pltpu.make_async_copy(w3_hbm, w3_v, sem_b),
             pltpu.make_async_copy(w2_hbm, w2_v, sem_b)]
    xs = [xcopy(i) for i in range(NB1)]
    for c in [xs[0]] + wk + xs[1:] + grp_a + grp_b:
        c.start()

    xs[0].wait()
    x0 = x_v[pl.ds(0, TM1), :]
    pks = []
    for s, (o, w) in enumerate(zip(offs, SLABS)):
        wk[s].wait()
        pks.append(_phi(_dot(x0, wk_v[:, pl.ds(o, w)])).astype(bf16))
        if s > 0:
            px_v[pl.ds(offs[s - 1], SLABS[s - 1]), :] = _dot_tn(pks[s - 1], x0)
    px_v[pl.ds(offs[-1], SLABS[-1]), :] = _dot_tn(pks[-1], x0)
    z0 = jnp.sum(jnp.concatenate(pks, axis=1).astype(f32), axis=0, keepdims=True)

    def p1(i, z):
        xcopy(i).wait()
        xi = x_v[pl.ds(pl.multiple_of(i * TM1, TM1), TM1), :]
        pk = _phi(_dot(xi, wk_v[...])).astype(bf16)
        px_v[...] += _dot_tn(pk, xi)
        return z + jnp.sum(pk.astype(f32), axis=0, keepdims=True)

    z = lax.fori_loop(1, NB1, p1, z0)

    for c in grp_a:
        c.wait()
    same_head = (lax.broadcasted_iota(jnp.int32, (128, 128), 0) // DH
                 == lax.broadcasted_iota(jnp.int32, (128, 128), 1) // DH)
    kvs = []
    for j in range(NJ + 1):
        if j < NJ:
            sl = slice(j * 128, (j + 1) * 128)
            kv = _dot(px_v[sl, :].astype(bf16), wv_v[:, sl])
            kvs.append(jnp.where(same_head, kv, 0.0).astype(bf16))
        if j > 0:
            sp = slice((j - 1) * 128, j * 128)
            m_v[sp, :] = _dot(kvs[j - 1], wo_v[sp, :]).astype(bf16)
        if j < NJ:
            zc_v[sl, :] = jnp.broadcast_to(z[:, sl], (128, 128)).T
    wqt_v[...] = wq_v[...].T
    for c in grp_b:
        c.wait()

    gw = gw_v[...].astype(f32).reshape(1, D)

    def ocopy(i, slot, n):
        cols = pl.ds(n * OW, OW)
        return pltpu.make_async_copy(out_v.at[slot, :, cols],
                                     out_hbm.at[pl.ds(pl.multiple_of(i * TM, TM), TM), cols],
                                     osems.at[slot])

    tiles = [[] for _ in range(NF)]
    for j in range(NJ):
        tiles[QPOS + j * (NF - QPOS) // NJ].append(j)

    def p2(i, carry):
        slot = i % 2

        @pl.when(i >= 2)
        def _():
            for n in range(OSPLIT):
                ocopy(i - 2, slot, n).wait()

        xi = x_v[pl.ds(pl.multiple_of(i * TM, TM), TM), :]
        g = _sigmoid(jnp.sum(xi.astype(f32) * gw, axis=-1, keepdims=True))
        og = 1.0 - g
        pqt, pqn, hs, acc = None, [], [], None
        for f in range(NF):
            if f == QPOS:
                pqt = _phi(_dot_nt(wqt_v[...], xi))
            fs = slice(f * TF, (f + 1) * TF)
            gate = _dot(xi, w1_v[:, fs])
            up = _dot(xi, w3_v[:, fs])
            if f > 0:
                d = _dot(hs[f - 1], w2_v[(f - 1) * TF:f * TF, :])
                acc = d if acc is None else acc + d
            for j in tiles[f]:
                pj = pqt[j * 128:(j + 1) * 128, :]
                zc = zc_v[j * 128:(j + 1) * 128, :]
                t = pj * jnp.concatenate([zc] * (TM // 128), axis=1)
                den = jnp.sum(t.reshape(128 // DH, DH, TM), axis=1, keepdims=True) + 1e-6
                r = pltpu.reciprocal(den, approx=False, full_range=False)
                pqn.append((pj.reshape(128 // DH, DH, TM) * r).reshape(128, TM).astype(bf16))
            hg = 0.5 * gate
            hs.append(((hg * jnp.tanh(hg) + hg) * (up * og)).astype(bf16))
        acc = acc + g * _dot_tn(jnp.concatenate(pqn, axis=0), m_v[...])
        for n in range(OSPLIT):
            cols = slice(n * OW, (n + 1) * OW)
            o = acc[:, cols] + _dot(hs[NF - 1], w2_v[(NF - 1) * TF:NF * TF, cols])
            out_v[slot, :, cols] = o.astype(bf16)
            ocopy(i, slot, n).start()
        return carry

    lax.fori_loop(0, NB, p2, None)
    for i in (NB - 2, NB - 1):
        for n in range(OSPLIT):
            ocopy(i, i % 2, n).wait()


@jax.jit
def pallas_gated_mix__linear_attn_block__glu_gated_swiglu__prompt_kernel(
    A_x: jax.Array,
    A_wqkv: jax.Array,
    A_wo: jax.Array,
    B_x: jax.Array,
    B_w1: jax.Array,
    B_w3: jax.Array,
    B_w2: jax.Array,
    gate_w: jax.Array,
):
    del B_x
    hbm = pl.BlockSpec(memory_space=pl.ANY)
    out = pl.pallas_call(
        _kernel,
        out_shape=jax.ShapeDtypeStruct((S, D), bf16),
        in_specs=[hbm] * 7,
        out_specs=hbm,
        scratch_shapes=[
            pltpu.VMEM((S, D), bf16),
            pltpu.VMEM((D, D), bf16),
            pltpu.VMEM((D, D), bf16),
            pltpu.VMEM((D, D), bf16),
            pltpu.VMEM((D, D), bf16),
            pltpu.VMEM((D, F), bf16),
            pltpu.VMEM((D, F), bf16),
            pltpu.VMEM((F, D), bf16),
            pltpu.VMEM((D,), bf16),
            pltpu.VMEM((D, D), f32),
            pltpu.VMEM((D, D), bf16),
            pltpu.VMEM((D, D), bf16),
            pltpu.VMEM((D, 128), f32),
            pltpu.VMEM((2, TM, D), bf16),
            pltpu.SemaphoreType.DMA((NB1 + len(SLABS) + 2,)),
            pltpu.SemaphoreType.DMA((2,)),
        ],
        compiler_params=pltpu.CompilerParams(vmem_limit_bytes=100 * 1024 * 1024),
    )(A_x.reshape(S, D), A_wqkv, A_wo, B_w1, B_w3, B_w2, gate_w)
    return out.reshape(1, S, D)
```

```python
import jax
import jax.numpy as jnp
from jax import lax
import jax.experimental.pallas as pl
import jax.experimental.pallas.tpu as pltpu

S, D, F, H = 2048, 1024, 3584, 32
DH = D // H
TM = 256
TF = 512
SLABS = (128, 128, 128, 128, 256, 256)
ORDER = (2, 4, 1, 3, 0, 6, 5)
HP = 3
APOS = 6
PXS = 4

NF = F // TF
NB = S // TM
NJ = D // 128
HM, HD, HF = TM // 2, D // 2, TF // 2
f32 = jnp.float32
bf16 = jnp.bfloat16
u32 = jnp.uint32
assert NF == NB - 1 and TF == HD


def _phi(t):
    return jnp.where(t > 0, t + 1.0, jnp.exp(t)) + 1e-6


def _dot(a, b):
    return jnp.dot(a, b, preferred_element_type=f32)


def _dot_tn(a, b):
    return lax.dot_general(a, b, (((0,), (0,)), ((), ())), preferred_element_type=f32)


def _dot_nt(a, b):
    return lax.dot_general(a, b, (((1,), (1,)), ((), ())), preferred_element_type=f32)


def _left(a11, a12, a21, a22):
    return [a11 + a22, a21 + a22, a11, a22, a11 + a12, a21 - a11, a12 - a22]


def _right(b11, b12, b21, b22):
    return [b11 + b22, b11, b12 - b22, b21 - b11, b22, b11 + b12, b21 + b22]


def _quads(v):
    r, c = v.shape[0] // 2, v.shape[1] // 2
    return v[:r, :c], v[:r, c:], v[r:, :c], v[r:, c:]


def _left2(a11, a12, a21, a22):
    return [t.astype(bf16) for v in _left(a11, a12, a21, a22) for t in _left(*_quads(v))]


def _combine(m):
    return (m[0] + m[3] - m[4] + m[6], m[2] + m[4], m[1] + m[3], m[0] - m[1] + m[2] + m[5])


def _assemble(m):
    c11, c12, c21, c22 = _combine(m)
    return jnp.concatenate([jnp.concatenate([c11, c12], axis=1), jnp.concatenate([c21, c22], axis=1)], axis=0)


def _words(t):
    return pltpu.bitcast(t, u32)


def _unwords(t):
    return pltpu.bitcast(t, bf16)


def _split_consts(t):
    ok = t[:8, :128] == t[:8, :128]
    return jnp.where(ok, u32(16), u32(0)), jnp.where(ok, u32(0xFFFF0000), u32(0))


def _rows_f32(w, sh, mk):
    return pltpu.bitcast(jnp.stack([w << sh, w & mk]), f32)


def _round_words(vals):
    u = pltpu.bitcast(jnp.stack(vals), u32) + u32(0x8000)
    return (u[:, 0] >> 16) | (u[:, 1] & u32(0xFFFF0000))


def _right_words(v, w):
    ops = _right(*v)
    if w is None:
        return _round_words(ops)
    p = _round_words([ops[0], ops[2], ops[3], ops[5], ops[6]])
    return jnp.concatenate([p[:1], w[0][None], p[1:3], w[1][None], p[3:]])


GROUPS = ((0, 1, 4), (2, 5), (3, 6))


def _right2_tile(quad, ts, dep, dst):
    sh, mk = (jnp.concatenate([c, c], axis=1) for c in _split_consts(dep))
    ws, vs = {}, {}
    for t in ts:
        qa, qb, sg = ((0, 3, 1), (0, None, 0), (1, 3, -1), (2, 0, -1), (3, None, 0), (0, 1, 1), (2, 3, 1))[t]
        for q in (qa, qb):
            if q is not None and q not in ws:
                ws[q] = quad(q)
                vs[q] = _rows_f32(ws[q], sh, mk)
        v = vs[qa] if qb is None else vs[qa] + vs[qb] if sg > 0 else vs[qa] - vs[qb]
        dst(t, _right_words((v[:, 0, :, :128], v[:, 0, :, 128:], v[:, 1, :, :128], v[:, 1, :, 128:]),
                            (ws[qa][0, :, :128], ws[qa][1, :, 128:]) if qb is None else None))


def _kernel(x_hbm, wqkv_hbm, wo_hbm, w1_hbm, w3_hbm, w2_hbm, gw_hbm, out_hbm,
            x_v, wq_v, wk_v, wv_v, wo_v, w1_v, w3_v, w2_v, gw_v,
            px_v, zc_v, out_v, b13_v, b2_v, bq_v, bm_v, sems, osems):
    s_wk = NB
    s_a = s_wk + len(SLABS)
    s_w2 = s_a + 1
    s_w13 = s_w2 + NF

    def xcopy(i):
        r = pl.ds(pl.multiple_of(i * TM, TM), TM)
        return pltpu.make_async_copy(x_hbm.at[r], x_v.at[r], sems.at[i])

    def w2copy(c):
        return pltpu.make_async_copy(w2_hbm.at[pl.ds(pl.multiple_of(c * TF, TF), TF)], w2_v.at[c], sems.at[s_w2 + c])

    def w13copy(c, half):
        cols = pl.ds(pl.multiple_of(c * TF + half * HF, HF), HF)
        return [pltpu.make_async_copy(src.at[:, cols], dst.at[c, :, pl.ds(half * HF, HF)], sems.at[s_w13 + 2 * c + half])
                for src, dst in ((w1_hbm, w1_v), (w3_hbm, w3_v))]

    offs = [sum(SLABS[:s]) for s in range(len(SLABS))]
    wk = [pltpu.make_async_copy(wqkv_hbm.at[:, pl.ds(D + o, w)], wk_v.at[:, pl.ds(o, w)], sems.at[s_wk + s])
          for s, (o, w) in enumerate(zip(offs, SLABS))]
    late = [pltpu.make_async_copy(wqkv_hbm.at[:, pl.ds(2 * D, D)], wv_v, sems.at[s_a]),
            pltpu.make_async_copy(wo_hbm, wo_v, sems.at[s_a]),
            pltpu.make_async_copy(wqkv_hbm.at[:, pl.ds(0, D)], wq_v, sems.at[s_a]),
            pltpu.make_async_copy(gw_hbm, gw_v, sems.at[s_a])]
    order = [xcopy(0)] + wk
    for i in range(1, NB):
        order += [xcopy(i), w2copy(i - 1)] + w13copy(i - 1, 0) + w13copy(i - 1, 1)
    for c in order + late:
        c.start()

    xcopy(0).wait()
    x0 = x_v[pl.ds(0, TM), :]
    pks = []
    for s, (o, w) in enumerate(zip(offs, SLABS)):
        wk[s].wait()
        pks.append(_phi(_dot(x0, wk_v[:, pl.ds(o, w)])).astype(bf16))
        if s > 0:
            px_v[pl.ds(offs[s - 1], SLABS[s - 1]), :] = _dot_tn(pks[s - 1], x0)
    px_v[pl.ds(offs[-1], SLABS[-1]), :] = _dot_tn(pks[-1], x0)
    z0 = jnp.sum(jnp.concatenate(pks, axis=1).astype(f32), axis=0, keepdims=True)

    def p1(i, z):
        c = i - 1
        xcopy(i).wait()
        w2copy(c).wait()
        xi = x_v[pl.ds(pl.multiple_of(i * TM, TM), TM), :]
        kf = _phi(_dot(xi, wk_v[...]))
        pk = kf.astype(bf16)

        w2w = _words(w2_v[c]).reshape(2, 2, 8, 8, D)
        ng = len(GROUPS)
        n2 = 8 * 2 * ng
        for n in range(n2):
            ts, r, cc = GROUPS[n % ng], n // (2 * ng), ((n // ng) % 2) * 128
            pos = n * NJ * 16 // n2
            dc, dr = (pos // 16) * 128, (pos % 16) * 16

            def quad2(q):
                col = (q % 2) * HD + cc
                blk = w2w[:, q // 2, r]
                return jnp.concatenate([blk[:, :, col:col + 128], blk[:, :, col + 256:col + 384]], axis=2)

            def put2(t, v):
                b2_v[c, t * 7:t * 7 + 7, r * 8:r * 8 + 8, cc:cc + 128] = v

            _right2_tile(quad2, ts, kf[dr:dr + 8, dc:dc + 128], put2)

        pw = D // PXS
        us = []
        for s in range(PXS):
            us.append(_dot_tn(pk, xi[:, s * pw:(s + 1) * pw]))
            px_v[:, s * pw:(s + 1) * pw] += us[s]

        n13 = 16 * 2 * ng
        for half in range(2):
            for cp in w13copy(c, half):
                cp.wait()
            w13w = [_words(src[c, ro:ro + HD, half * HF:(half + 1) * HF]).reshape(2, 16, 8, HF)
                    for src, ro in ((w1_v, 0), (w3_v, 0), (w1_v, HD), (w3_v, HD))]
            for n in range(half * n13 // 2, (half + 1) * n13 // 2):
                ts, r = GROUPS[n % ng], (n // ng) % 16
                pos = n * (PXS * 64 - 8) // n13
                dr = (pos % 64) * 16

                def put13(t, v):
                    b13_v[c, t * 7:t * 7 + 7, r * 8:r * 8 + 8, half * 128:half * 128 + 128] = v

                _right2_tile(lambda q: w13w[q][:, r], ts, us[pos // 64][dr:dr + 8, pw - 128:], put13)
        return z + jnp.sum(pk.astype(f32), axis=0, keepdims=True)

    z = lax.fori_loop(1, NB, p1, z0)

    for c in late:
        c.wait()
    same_head = (lax.broadcasted_iota(jnp.int32, (128, 128), 0) // DH
                 == lax.broadcasted_iota(jnp.int32, (128, 128), 1) // DH)
    jorder = [j + h * NJ // 2 for j in range(NJ // 2) for h in range(2)]
    kvf, kvb, ms = [], {}, {}
    for n in range(NJ + 1):
        if n < NJ:
            sl = slice(jorder[n] * 128, (jorder[n] + 1) * 128)
            kvf.append(_dot(px_v[sl, :].astype(bf16), wv_v[:, sl]))
            kvb[jorder[n]] = jnp.where(same_head, kvf[n], 0.0).astype(bf16)
        if n > 0:
            j = jorder[n - 1]
            ms[j] = _dot(kvb[j], wo_v[j * 128:(j + 1) * 128, :])
            if j >= NJ // 2:
                lo, hi = ms[j - NJ // 2], ms[j]
                for t, v in enumerate(_right(lo[:, :HD], lo[:, HD:], hi[:, :HD], hi[:, HD:])):
                    bm_v[t, (j - NJ // 2) * 64:(j - NJ // 2 + 1) * 64, :] = _words(v.astype(bf16))
        if n < NJ:
            zc_v[sl, :] = jnp.broadcast_to(z[:, sl], (128, 128)).T
    wqw = [_words(q.T) for q in _quads(wq_v[...])]
    nq = (HD // 16) * (HD // 128)
    for n in range(nq):
        r, cc = (n // 4) * 8, (n % 4) * 128
        pos = n * NJ * 8 // nq
        sh, mk = _split_consts(kvf[pos // 8][(pos % 8) * 16:(pos % 8) * 16 + 8, :])
        w = [q[r:r + 8, cc:cc + 128] for q in wqw]
        bq_v[:, r:r + 8, cc:cc + 128] = _right_words([_rows_f32(q, sh, mk) for q in w], (w[0], w[3]))

    gw = gw_v[...].astype(f32).reshape(1, D)

    def ocopy(i, slot, q):
        rows, cols = (q // 2) * HM, pl.ds((q % 2) * HD, HD)
        return pltpu.make_async_copy(out_v.at[slot, pl.ds(rows, HM), cols],
                                     out_hbm.at[pl.ds(pl.multiple_of(i * TM + rows, HM), HM), cols],
                                     osems.at[slot])

    pairs = [[] for _ in range(NF)]
    for j in range(NJ // 2):
        pairs[j * (APOS + 1) // (NJ // 2)].append(j)

    def p2(i, carry):
        slot = i % 2

        @pl.when(i >= 2)
        def _():
            for q in range(4):
                ocopy(i - 2, slot, q).wait()

        xf = x_v[pl.ds(pl.multiple_of(i * TM, TM), TM), :].astype(f32)
        xa2 = _left2(*_quads(xf))
        g = 0.5 * jnp.tanh(0.5 * jnp.sum(xf * gw, axis=-1, keepdims=True)) + 0.5
        og = 1.0 - g
        grow = jnp.broadcast_to(g, (TM, 128)).T[:1, :].reshape(1, 1, TM)

        q11, q12, q21, q22 = _combine([_dot_nt(_unwords(bq_v[t]), a.astype(bf16))
                                       for t, a in enumerate(_left(*_quads(xf)))])
        pqt = jnp.concatenate([_phi(jnp.concatenate([q11, q21], axis=1)),
                               _phi(jnp.concatenate([q12, q22], axis=1))], axis=0)

        def normalised(j):
            pj = pqt[j * 128:(j + 1) * 128, :]
            zc = zc_v[j * 128:(j + 1) * 128, :]
            t = pj * jnp.concatenate([zc] * (TM // 128), axis=1)
            den = jnp.sum(t.reshape(128 // DH, DH, TM), axis=1, keepdims=True) + 1e-6
            r = pltpu.reciprocal(den, approx=False, full_range=False) * grow
            return (pj.reshape(128 // DH, DH, TM) * r).reshape(128, TM)

        def act(gate, up, o):
            hg = 0.5 * gate
            return (hg * jnp.tanh(hg) + hg) * (up * o)

        pqn, ha, att, dacc = [], None, None, [None] * 49
        for f in range(NF + 1):
            m = [None] * 7

            def gate_up(ts):
                for t in ts:
                    e = [None] * 7
                    for u in ORDER:
                        e[u] = _dot(xa2[t * 7 + u], _unwords(b13_v[f, t * 7 + u]))
                    m[t] = _assemble(e)

            if f < NF:
                gate_up(ORDER[:HP])
            if 0 < f < NF:
                for t in range(49):
                    d = _dot(ha[t], _unwords(b2_v[f - 1, t]))
                    dacc[t] = d if dacc[t] is None else dacc[t] + d
            if f == NF:
                def put(q, v):
                    out_v[slot, (q // 2) * HM:(q // 2 + 1) * HM, (q % 2) * HD:(q % 2 + 1) * HD] = v.astype(bf16)
                    ocopy(i, slot, q).start()

                for t in ORDER:
                    e = [None] * 7
                    for u in ORDER:
                        e[u] = dacc[t * 7 + u] + _dot(ha[t * 7 + u], _unwords(b2_v[f - 1, t * 7 + u]))
                    m[t] = att[t] + _assemble(e)
                    if t == 4:
                        put(1, m[2] + m[4])
                    if t == 3:
                        put(2, m[1] + m[3])
                    if t == 6:
                        put(0, m[0] + m[3] - m[4] + m[6])
                    if t == 5:
                        put(3, m[0] - m[1] + m[2] + m[5])
            else:
                gate_up(ORDER[HP:])
                for j in pairs[f]:
                    lo, hi = normalised(j), normalised(j + NJ // 2)
                    pqn.append([v.astype(bf16) for v in _left(lo[:, :HM], hi[:, :HM], lo[:, HM:], hi[:, HM:])])
                gate1, up1, gate2, up2 = _combine(m)
                h1, h2 = act(gate1, up1, og[:HM]), act(gate2, up2, og[HM:])
                ha = _left2(h1[:, :HF], h1[:, HF:], h2[:, :HF], h2[:, HF:])
                if f == APOS:
                    att = [_dot_tn(jnp.concatenate([p[t] for p in pqn], axis=0), _unwords(bm_v[t])) for t in range(7)]
        return carry

    lax.fori_loop(0, NB, p2, None)
    for i in (NB - 2, NB - 1):
        for q in range(4):
            ocopy(i, i % 2, q).wait()


@jax.jit
def pallas_gated_mix__linear_attn_block__glu_gated_swiglu__prompt_kernel(
    A_x: jax.Array,
    A_wqkv: jax.Array,
    A_wo: jax.Array,
    B_x: jax.Array,
    B_w1: jax.Array,
    B_w3: jax.Array,
    B_w2: jax.Array,
    gate_w: jax.Array,
):
    del B_x
    hbm = pl.BlockSpec(memory_space=pl.ANY)
    out = pl.pallas_call(
        _kernel,
        out_shape=jax.ShapeDtypeStruct((S, D), bf16),
        in_specs=[hbm] * 7,
        out_specs=hbm,
        scratch_shapes=[
            pltpu.VMEM((S, D), bf16),
            pltpu.VMEM((D, D), bf16),
            pltpu.VMEM((D, D), bf16),
            pltpu.VMEM((D, D), bf16),
            pltpu.VMEM((D, D), bf16),
            pltpu.VMEM((NF, D, TF), bf16),
            pltpu.VMEM((NF, D, TF), bf16),
            pltpu.VMEM((NF, TF, D), bf16),
            pltpu.VMEM((D,), bf16),
            pltpu.VMEM((D, D), f32),
            pltpu.VMEM((D, 128), f32),
            pltpu.VMEM((2, TM, D), bf16),
            pltpu.VMEM((NF, 49, HD // 4, TF // 2), u32),
            pltpu.VMEM((NF, 49, TF // 8, D // 4), u32),
            pltpu.VMEM((7, HD // 2, HD), u32),
            pltpu.VMEM((7, HD // 2, HD), u32),
            pltpu.SemaphoreType.DMA((NB + len(SLABS) + 1 + 3 * NF,)),
            pltpu.SemaphoreType.DMA((2,)),
        ],
        compiler_params=pltpu.CompilerParams(
            vmem_limit_bytes=124 * 1024 * 1024,
            flags={"XLA_TPU_RESCHEDULE_DMA_DONES": True},
        ),
    )(A_x.reshape(S, D), A_wqkv, A_wo, B_w1, B_w3, B_w2, gate_w)
    return out.reshape(1, S, D)
```
